```python
import os as _os
_os.environ.setdefault("JAX_PLATFORMS", "cpu")
import jax
import jax.numpy as jnp

def _softmax(x, axis=-1):
    return jax.nn.softmax(x, axis=axis)
def _gelu(x):
    return jax.nn.gelu(x, approximate=True)
def _silu(x):
    return jax.nn.silu(x)
def _sigmoid(x):
    return jax.nn.sigmoid(x)
def _layernorm(x, axis=-1, eps=1e-5):
    m = jnp.mean(x, axis=axis, keepdims=True)
    v = jnp.var(x, axis=axis, keepdims=True)
    return (x - m) / jnp.sqrt(v + eps)
def _scatter_add(tgt, idx, src, axis=0):
    return tgt.at[idx].add(src)
def _segment_sum(src, seg, n):
    return jax.ops.segment_sum(src, seg, n)
class _Rng:
    def __init__(self, key):
        self._k = key
    def _next(self):
        self._k, sub = jax.random.split(self._k)
        return sub
    def normal(self, shape):
        return jax.random.normal(self._next(), shape, dtype=jnp.bfloat16)
    def randint(self, lo, hi, shape):
        return jax.random.randint(self._next(), shape, lo, hi, dtype=jnp.int32)
    def uniform(self, shape, lo=0.0, hi=1.0):
        return jax.random.uniform(self._next(), shape, jnp.bfloat16, lo, hi)
    def permutation(self, n):
        return jax.random.permutation(self._next(), n)


kernel_name = 'sequential_preLN__mha_block__mixer_token_mlp__prompt'

def setup_inputs():
    _rng = _Rng(jax.random.key(int.from_bytes(__import__("os").urandom(4), "little")))
    _w = (lambda a: (lambda t: t.astype(jnp.bfloat16) if jnp.issubdtype(t.dtype, jnp.floating) else t)(jnp.asarray(a)))
    def _A_setup():
        B, S, D, H = 1, 2048, 448, 16
        return {
            "x": _w((lambda *s: _rng.normal(s) * 0.05)(B, S, D)),
            "wqkv": _w((lambda *s: _rng.normal(s) * 0.05)(D, 3 * D)),
            "wo": _w((lambda *s: _rng.normal(s) * 0.05)(D, D)),
        }
    _A_in = _A_setup()

    def _B_setup():
        B, S, D, F = 1, 2048, 448, 1792
        return {
            "x": _w((lambda *s: _rng.normal(s) * 0.05)(B, S, D)),
            "w1": _w((lambda *s: _rng.normal(s) * 0.2)(S, F) * (S ** -0.5)),
            "b1": _w((lambda *s: _rng.normal(s) * 0.2)(F) * 0.02),
            "w2": _w((lambda *s: _rng.normal(s) * 0.2)(F, S) * (F ** -0.5)),
            "b2": _w((lambda *s: _rng.normal(s) * 0.05)(S) * 0.02),
        }
    _B_in = _B_setup()

    return {
        "A_x": _A_in["x"],
        "A_wqkv": _A_in["wqkv"],
        "A_wo": _A_in["wo"],
        "B_x": _B_in["x"],
        "B_w1": _B_in["w1"],
        "B_b1": _B_in["b1"],
        "B_w2": _B_in["w2"],
        "B_b2": _B_in["b2"],
    }

def reference(A_x, A_wqkv, A_wo, B_x, B_w1, B_b1, B_w2, B_b2):
    def _A_ref(x, wqkv, wo):
        B, S, D = x.shape
        H = 16
        Dh = D // H
        qkv = (lambda x, *d: x.transpose(*d))((x @ wqkv).reshape(B, S, 3, H, Dh), 2, 0, 3, 1, 4)
        q, k, v = qkv[0], qkv[1], qkv[2]
        scores = jnp.einsum("bhqd,bhkd->bhqk", q, k) * (Dh ** -0.5)
        p = _softmax(scores, axis=-1)
        o = jnp.einsum("bhqk,bhkd->bhqd", p, v)
        return (lambda x, *d: x.transpose(*d))(o, 0, 2, 1, 3).reshape(B, S, D) @ wo

    def _B_ref(x, w1, b1, w2, b2):
        B, S, D = x.shape
        h = _layernorm(x, axis=-1)
        u = jnp.einsum("bsd,sf->bdf", h, w1) + b1
        u = _gelu(u)
        y = jnp.einsum("bdf,fs->bds", u, w2) + b2
        return (lambda x, *d: x.transpose(*d))(y, 0, 2, 1)

    x = A_x
    h = x + _A_ref(_layernorm(x, axis=-1), A_wqkv, A_wo)
    h2 = h + _B_ref(_layernorm(h, axis=-1), B_w1, B_b1, B_w2, B_b2)
    return h2
```

```python
import jax
import jax.numpy as jnp
import numpy as np
from jax import lax
import jax.experimental.pallas as pl
import jax.experimental.pallas.tpu as pltpu

_H = 16
_HP = 32
_EPS = 1e-5
_BQ = 2048
_BK = 128
_AU = 1
_CB = 512
_FB = 512
_SB = 512
_LO = 2.0 ** -30
_HI = 2.0 ** 60
_BF = jnp.bfloat16
_F32 = jnp.float32


def _dot(a, b):
    return jnp.dot(a, b, preferred_element_type=_F32)


def _layernorm_t(x):
    xc = x - jnp.mean(x, axis=0, keepdims=True)
    v = jnp.mean(xc * xc, axis=0, keepdims=True)
    return xc * lax.rsqrt(v + _EPS)


def _pad_heads(t, dh, extra):
    return [jnp.concatenate([t[h * dh:(h + 1) * dh], extra], axis=0) for h in range(_H)]


def _kernel(x_ref, wqkv_ref, wo_ref, b1_ref, b2_ref, w1_hbm, w2_hbm, o_hbm,
            w1_v, w2_v, res_v, h_v, qt_v, k_v, vt_v, ot_v, g_v, o_v, sems):
    D, S = x_ref.shape
    F = w1_v.shape[1]
    Dh = D // _H
    PAD = _HP - Dh

    w1_cp = pltpu.make_async_copy(w1_hbm, w1_v, sems.at[0])
    w2_cp = pltpu.make_async_copy(w2_hbm, w2_v, sems.at[1])
    w1_cp.start()
    w2_cp.start()

    w_t = wqkv_ref[...].astype(_F32).T.astype(_BF)
    wq_t, wk_t, wv_t = w_t[0:D], w_t[D:2 * D], w_t[2 * D:3 * D]
    one_row = lax.broadcasted_iota(jnp.int32, (PAD, _CB), 0) == 0
    e0 = one_row.astype(_F32)
    kmax = [None] * _H
    for c in range(S // _CB):
        sl = pl.ds(c * _CB, _CB)
        hb = _layernorm_t(x_ref[:, sl].astype(_F32)).astype(_BF)
        h_v[:, sl] = hb
        ks = _pad_heads(_dot(wk_t, hb), Dh, e0)
        for h in range(_H):
            n2 = jnp.sum(ks[h] * ks[h], axis=0, keepdims=True)
            kmax[h] = n2 if c == 0 else jnp.maximum(kmax[h], n2)
        for t in range(_H // 4):
            kt = jnp.concatenate(ks[4 * t:4 * t + 4], axis=0).T.astype(_BF)
            for j in range(4):
                k_v[4 * t + j, sl, :] = kt[:, j * _HP:(j + 1) * _HP]
        for h, v in enumerate(_pad_heads(_dot(wv_t, hb), Dh, e0)):
            vt_v[pl.ds(h * _HP, _HP), sl] = v.astype(_BF)
    kmax = [jnp.max(m, axis=1, keepdims=True) for m in kmax]
    qscale = float(Dh ** -0.5 * np.log2(np.e))
    zpad = jnp.zeros((PAD, _CB), _F32)
    shift_row = lax.broadcasted_iota(jnp.int32, (_HP, _CB), 0) == Dh
    for c in range(S // _CB):
        sl = pl.ds(c * _CB, _CB)
        for h, q in enumerate(_pad_heads(_dot(wq_t, h_v[:, sl]) * qscale, Dh, zpad)):
            bound = jnp.sqrt(jnp.sum(q * q, axis=0, keepdims=True) * kmax[h])
            qt_v[pl.ds(h * _HP, _HP), sl] = jnp.where(shift_row, -bound, q).astype(_BF)

    def step_slices(i, bq):
        h = i // (S // bq)
        return (h, pl.ds(pl.multiple_of(h * _HP, _HP), _HP),
                pl.ds(pl.multiple_of((i % (S // bq)) * bq, bq), bq))

    def attn_step(i, safe):
        h, hs, qs = step_slices(i, _BQ)
        q = qt_v[hs, qs]
        n = S // _BK
        acc = None
        s = _dot(k_v[h, pl.ds(0, _BK), :], q)
        for c in range(n):
            s_next = _dot(k_v[h, pl.ds((c + 1) * _BK, _BK), :], q) if c + 1 < n else None
            pv = _dot(vt_v[hs, pl.ds(c * _BK, _BK)], jnp.exp2(s).astype(_BF))
            acc = pv if acc is None else acc + pv
            s = s_next
        l = acc[Dh:Dh + 1, :]
        ot_v[hs, qs] = (acc / l).astype(_BF)
        return jnp.where((l >= _LO) & (l <= _HI), safe, 0.0)

    safe = lax.fori_loop(0, _H * S // _BQ, attn_step, jnp.ones((1, _BQ), _F32), unroll=_AU)

    @pl.when(jnp.min(safe) < 0.5)
    def _():
        bq, bk = 256, 256
        keep = lax.broadcasted_iota(jnp.int32, (_HP, bq), 0) < Dh

        def exact_step(i, carry):
            h, hs, qs = step_slices(i, bq)
            q = qt_v[hs, qs]
            q = jnp.where(keep, q, jnp.zeros_like(q))

            def chunk(c, mc):
                m, acc = mc
                ks = pl.ds(pl.multiple_of(c * bk, bk), bk)
                s = _dot(k_v[h, ks, :], q)
                m_new = jnp.maximum(m, jnp.max(s, axis=0, keepdims=True))
                pv = _dot(vt_v[hs, ks], jnp.exp2(s - m_new).astype(_BF))
                return m_new, acc * jnp.exp2(m - m_new) + pv

            init = (jnp.full((1, bq), -jnp.inf, _F32), jnp.zeros((_HP, bq), _F32))
            _, acc = lax.fori_loop(0, S // bk, chunk, init)
            ot_v[hs, qs] = (acc / acc[Dh:Dh + 1, :]).astype(_BF)
            return carry

        lax.fori_loop(0, _H * S // bq, exact_step, 0)

    wo = wo_ref[...].astype(_F32)
    wo = jnp.concatenate(_pad_heads(wo, Dh, jnp.zeros((PAD, D), _F32)), axis=0)
    wo_t = wo.T.astype(_BF)
    for c in range(S // _CB):
        sl = pl.ds(c * _CB, _CB)
        hh = x_ref[:, sl].astype(_F32) + _dot(wo_t, ot_v[:, sl])
        res_v[:, sl] = hh
        h_v[:, sl] = _layernorm_t(hh).astype(_BF)

    w1_cp.wait()
    for lo in range(0, F, _FB):
        sl = pl.ds(lo, min(_FB, F - lo))
        u = _dot(h_v[...], w1_v[:, sl]) + b1_ref[:, sl].astype(_F32)
        g_v[:, sl] = jax.nn.gelu(u, approximate=True).astype(_BF)
    w2_cp.wait()
    cps = []
    for c in range(S // _SB):
        sl = pl.ds(c * _SB, _SB)
        y = _dot(g_v[...], w2_v[:, sl]) + b2_ref[:, sl].astype(_F32) + res_v[:, sl]
        o_v[:, sl] = y.astype(_BF)
        cps.append(pltpu.make_async_copy(o_v.at[:, sl], o_hbm.at[:, sl], sems.at[2 + c]))
        cps[-1].start()
    for cp in cps:
        cp.wait()


@jax.jit
def pallas_sequential_preLN__mha_block__mixer_token_mlp__prompt_kernel(
    A_x: jax.Array,
    A_wqkv: jax.Array,
    A_wo: jax.Array,
    B_x: jax.Array,
    B_w1: jax.Array,
    B_b1: jax.Array,
    B_w2: jax.Array,
    B_b2: jax.Array,
):
    del B_x
    B, S, D = A_x.shape
    F = B_w1.shape[1]
    E = _H * _HP
    vmem = pl.BlockSpec(memory_space=pltpu.VMEM)
    hbm = pl.BlockSpec(memory_space=pl.ANY)
    out = pl.pallas_call(
        _kernel,
        out_shape=jax.ShapeDtypeStruct((D, S), A_x.dtype),
        in_specs=[vmem] * 5 + [hbm] * 2,
        out_specs=hbm,
        scratch_shapes=[
            pltpu.VMEM((S, F), _BF),
            pltpu.VMEM((F, S), _BF),
            pltpu.VMEM((D, S), _F32),
            pltpu.VMEM((D, S), _BF),
            pltpu.VMEM((E, S), _BF),
            pltpu.VMEM((_H, S, _HP), _BF),
            pltpu.VMEM((E, S), _BF),
            pltpu.VMEM((E, S), _BF),
            pltpu.VMEM((D, F), _BF),
            pltpu.VMEM((D, S), _BF),
            pltpu.SemaphoreType.DMA((2 + S // _SB,)),
        ],
        compiler_params=pltpu.CompilerParams(vmem_limit_bytes=100 * 1024 * 1024),
    )(A_x.reshape(S, D).T, A_wqkv, A_wo, B_b1.reshape(1, F), B_b2.reshape(1, S), B_w1, B_w2)
    return out.T.reshape(B, S, D)
```

```python
import jax
import jax.numpy as jnp
import numpy as np
from jax import lax
import jax.experimental.pallas as pl
import jax.experimental.pallas.tpu as pltpu

_H = 16
_HP = 32
_EPS = 1e-5
_BQ = 2048
_BK = 512
_AU = 4
_CB = 128
_OB = 512
_FB = 896
_SP = (256,) * 7 + (128, 128)
_LO = 2.0 ** -30
_HI = 2.0 ** 30
_XP = (512, 1024, 512)
_BF = jnp.bfloat16
_F32 = jnp.float32


def _dot(a, b):
    return jnp.dot(a, b, preferred_element_type=_F32)


def _layernorm_t(x):
    mean = jnp.mean(x, axis=0, keepdims=True)
    xc = x - mean
    rstd = lax.rsqrt(jnp.mean(xc * xc, axis=0, keepdims=True) + _EPS)
    return xc * rstd, mean, rstd


def _pad_heads(t, dh, extra):
    return [jnp.concatenate([t[h * dh:(h + 1) * dh], extra], axis=0) for h in range(_H)]


def _kernel(x_hbm, wqkv_hbm, wo_hbm, b1_ref, b2_ref, w1_hbm, w2_hbm, o_hbm,
            x_ref, wv_ref, wqk_ref, wo_ref, wo_v, w1_v, w2_v, res_v, h_v, qt_v, k_v, vt_v, ot_v, g_v, o_v, sems):
    D, S = x_ref.shape
    F = w1_v.shape[1]
    Dh = D // _H
    PAD = _HP - Dh

    copies = [(wqkv_hbm.at[:, pl.ds(2 * D, D)], wv_ref)]
    x_parts = [pl.ds(sum(_XP[:i]), n) for i, n in enumerate(_XP)]
    copies += [(x_hbm.at[:, p], x_ref.at[:, p]) for p in x_parts]
    copies += [(wqkv_hbm.at[:, pl.ds(0, wqk_ref.shape[1])], wqk_ref),
               (wo_hbm, wo_ref), (w1_hbm, w1_v), (w2_hbm, w2_v)]
    copies = [pltpu.make_async_copy(a, b, sems.at[i]) for i, (a, b) in enumerate(copies)]
    wv_cp, x_cps, (wqk_cp, wo_cp, w1_cp, w2_cp) = copies[0], copies[1:-4], copies[-4:]
    for cp in (wv_cp, *x_cps, wqk_cp, wo_cp):
        cp.start()

    def project_v(part):
        for lo in range(part.start, part.start + part.size, _CB):
            sl = pl.ds(lo, _CB)
            x = x_ref[:, sl]
            raw = _dot(wv_t, x)
            hn, mean, rstd = _layernorm_t(x.astype(_F32))
            h_v[:, sl] = hn.astype(_BF)
            for h, v in enumerate(_pad_heads((raw - wv_sum * mean) * rstd, Dh, e0)):
                vt_v[pl.ds(h * _HP, _HP), sl] = v.astype(_BF)

    e0 = (lax.broadcasted_iota(jnp.int32, (PAD, _CB), 0) == 0).astype(_F32)
    wv_cp.wait()
    wv_t = wv_ref[...].T
    wv_sum = jnp.broadcast_to(jnp.sum(wv_t.astype(_F32), axis=1, keepdims=True), (D, _CB))
    x_cps[0].wait()
    project_v(x_parts[0])
    x_cps[1].wait()
    project_v(x_parts[1])
    x_cps[2].wait()
    wqk_cp.wait()
    wqk_t = wqk_ref[...].T
    wq_t, wk_t = wqk_t[0:D], wqk_t[D:2 * D]
    project_v(x_parts[2])
    kmax = [None] * _H
    for c in range(S // _CB):
        sl = pl.ds(c * _CB, _CB)
        ks = _pad_heads(_dot(wk_t, h_v[:, sl]), Dh, e0)
        for h in range(_H):
            n2 = jnp.sum(ks[h] * ks[h], axis=0, keepdims=True)
            kmax[h] = n2 if c == 0 else jnp.maximum(kmax[h], n2)
            k_v[pl.ds(h * _HP, _HP), sl] = ks[h].astype(_BF)
    kmax = [jnp.max(m, axis=1, keepdims=True) for m in kmax]
    wo_cp.wait()
    wo = _pad_heads(wo_ref[...].astype(_F32), Dh, jnp.zeros((PAD, D), _F32))
    wo_v[...] = jnp.concatenate(wo, axis=0).astype(_BF).T
    qscale = float(Dh ** -0.5 * np.log2(np.e))
    zpad = jnp.zeros((PAD, _CB), _F32)
    shift_row = lax.broadcasted_iota(jnp.int32, (_HP, _CB), 0) == Dh
    for c in range(S // _CB):
        sl = pl.ds(c * _CB, _CB)
        for h, q in enumerate(_pad_heads(_dot(wq_t, h_v[:, sl]) * qscale, Dh, zpad)):
            bound = jnp.sqrt(jnp.sum(q * q, axis=0, keepdims=True) * kmax[h])
            qt_v[pl.ds(h * _HP, _HP), sl] = jnp.where(shift_row, -bound, q).astype(_BF)

    def scores(hs, ks, q):
        return _dot(k_v[hs, ks].T, q)

    def step_slices(i, bq):
        h = i // (S // bq)
        return (pl.ds(pl.multiple_of(h * _HP, _HP), _HP),
                pl.ds(pl.multiple_of((i % (S // bq)) * bq, bq), bq))

    def attn_step(i, safe):
        hs, qs = step_slices(i, _BQ)
        q = qt_v[hs, qs]
        n = S // _BK
        acc = None
        s = scores(hs, pl.ds(0, _BK), q)
        for c in range(n):
            s_next = scores(hs, pl.ds((c + 1) * _BK, _BK), q) if c + 1 < n else None
            pv = _dot(vt_v[hs, pl.ds(c * _BK, _BK)], jnp.exp2(s).astype(_BF))
            acc = pv if acc is None else acc + pv
            s = s_next
        l = acc[Dh:Dh + 1, :]
        ot_v[hs, qs] = (acc / l).astype(_BF)
        return jnp.where((l >= _LO) & (l <= _HI), safe, 0.0)

    w1_cp.start()
    w2_cp.start()
    safe = lax.fori_loop(0, _H * S // _BQ, attn_step, jnp.ones((1, _BQ), _F32), unroll=_AU)

    @pl.when(jnp.min(safe) < 0.5)
    def _():
        bq, bk = 256, 256
        keep = lax.broadcasted_iota(jnp.int32, (_HP, bq), 0) < Dh

        def exact_step(i, carry):
            hs, qs = step_slices(i, bq)
            q = qt_v[hs, qs]
            q = jnp.where(keep, q, jnp.zeros_like(q))

            def chunk(c, mc):
                m, acc = mc
                ks = pl.ds(pl.multiple_of(c * bk, bk), bk)
                s = scores(hs, ks, q)
                m_new = jnp.maximum(m, jnp.max(s, axis=0, keepdims=True))
                pv = _dot(vt_v[hs, ks], jnp.exp2(s - m_new).astype(_BF))
                return m_new, acc * jnp.exp2(m - m_new) + pv

            init = (jnp.full((1, bq), -jnp.inf, _F32), jnp.zeros((_HP, bq), _F32))
            _, acc = lax.fori_loop(0, S // bk, chunk, init)
            ot_v[hs, qs] = (acc / acc[Dh:Dh + 1, :]).astype(_BF)
            return carry

        lax.fori_loop(0, _H * S // bq, exact_step, 0)

    w1_cp.wait()
    w2_cp.wait()
    for c in range(S // _OB):
        sl = pl.ds(c * _OB, _OB)
        hh = x_ref[:, sl].astype(_F32) + _dot(wo_v[...], ot_v[:, sl])
        res_v[:, sl] = hh
        h_v[:, sl] = _layernorm_t(hh)[0].astype(_BF)

    b1 = b1_ref[...].astype(_F32).reshape(1, F)
    b2 = b2_ref[...].astype(_F32).reshape(1, S)
    for lo in range(0, F, _FB):
        sl = pl.ds(lo, min(_FB, F - lo))
        u = _dot(h_v[...], w1_v[:, sl]) + b1[:, sl.start:sl.start + sl.size]
        g_v[:, sl] = jax.nn.gelu(u, approximate=True).astype(_BF)
    cps = []
    for c, width in enumerate(_SP):
        sl = pl.ds(sum(_SP[:c]), width)
        y = _dot(g_v[...], w2_v[:, sl]) + b2[:, sl.start:sl.start + sl.size] + res_v[:, sl]
        o_v[:, sl] = y.astype(_BF)
        cps.append(pltpu.make_async_copy(o_v.at[:, sl], o_hbm.at[:, sl], sems.at[len(copies) + c]))
        cps[-1].start()
    for cp in cps:
        cp.wait()


@jax.jit
def pallas_sequential_preLN__mha_block__mixer_token_mlp__prompt_kernel(
    A_x: jax.Array,
    A_wqkv: jax.Array,
    A_wo: jax.Array,
    B_x: jax.Array,
    B_w1: jax.Array,
    B_b1: jax.Array,
    B_w2: jax.Array,
    B_b2: jax.Array,
):
    del B_x
    B, S, D = A_x.shape
    F = B_w1.shape[1]
    E = _H * _HP
    vmem = pl.BlockSpec(memory_space=pltpu.VMEM)
    hbm = pl.BlockSpec(memory_space=pl.ANY)
    out = pl.pallas_call(
        _kernel,
        out_shape=jax.ShapeDtypeStruct((D, S), A_x.dtype),
        in_specs=[hbm] * 3 + [vmem] * 2 + [hbm] * 2,
        out_specs=hbm,
        scratch_shapes=[
            pltpu.VMEM((D, S), _BF),
            pltpu.VMEM((D, D), _BF),
            pltpu.VMEM((D, pl.cdiv(2 * D, 128) * 128), _BF),
            pltpu.VMEM((D, D), _BF),
            pltpu.VMEM((D, E), _BF),
            pltpu.VMEM((S, F), _BF),
            pltpu.VMEM((F, S), _BF),
            pltpu.VMEM((D, S), _F32),
            pltpu.VMEM((D, S), _BF),
            pltpu.VMEM((E, S), _BF),
            pltpu.VMEM((E, S), _BF),
            pltpu.VMEM((E, S), _BF),
            pltpu.VMEM((E, S), _BF),
            pltpu.VMEM((D, F), _BF),
            pltpu.VMEM((D, S), _BF),
            pltpu.SemaphoreType.DMA((5 + len(_XP) + len(_SP),)),
        ],
        compiler_params=pltpu.CompilerParams(vmem_limit_bytes=100 * 1024 * 1024),
    )(A_x.reshape(S, D).T, A_wqkv, A_wo, B_b1, B_b2, B_w1, B_w2)
    return out.T.reshape(B, S, D)
```
